```python
import jax
import jax.numpy as jnp

def _softmax(x, axis=-1):
    return jax.nn.softmax(x, axis=axis)

def _gelu(x):
    return jax.nn.gelu(x, approximate=True)

def _silu(x):
    return jax.nn.silu(x)

def _sigmoid(x):
    return jax.nn.sigmoid(x)

def _layernorm(x, axis=-1, eps=1e-05):
    m = jnp.mean(x, axis=axis, keepdims=True)
    v = jnp.var(x, axis=axis, keepdims=True)
    return (x - m) / jnp.sqrt(v + eps)

def _scatter_add(tgt, idx, src, axis=0):
    return tgt.at[idx].add(src)

def _segment_sum(src, seg, n):
    return jax.ops.segment_sum(src, seg, n)

class _Rng:

    def __init__(self, key):
        self._k = key

    def _next(self):
        self._k, sub = jax.random.split(self._k)
        return sub

    def normal(self, shape):
        return jax.random.normal(self._next(), shape, dtype=jnp.bfloat16)

    def randint(self, lo, hi, shape):
        return jax.random.randint(self._next(), shape, lo, hi, dtype=jnp.int32)

    def uniform(self, shape, lo=0.0, hi=1.0):
        return jax.random.uniform(self._next(), shape, jnp.bfloat16, lo, hi)

    def permutation(self, n):
        return jax.random.permutation(self._next(), n)
kernel_name = 'adaLN_cond__gqa_block_cached__moe_arch_mod__decode'

def setup_inputs():
    _rng = _Rng(jax.random.key(int.from_bytes(__import__("os").urandom(4), "little")))
    _w = lambda a: (lambda t: t.astype(jnp.bfloat16) if jnp.issubdtype(t.dtype, jnp.floating) else t)(jnp.asarray(a))

    def _A_setup():
        B, Sq, D = (4, 1, 512)
        Hq, Hkv, Sk, Dh = (32, 32, 8192, 128)
        assert Hq % Hkv == 0, (Hq, Hkv)
        return {'x': _w((lambda *s: _rng.normal(s) * 0.05)(B, Sq, D)), 'k_cache': _w((lambda *s: _rng.normal(s) * 0.05)(B, Hkv, Sk, Dh)), 'v_cache': _w((lambda *s: _rng.normal(s) * 0.05)(B, Hkv, Sk, Dh)), 'wq': _w((lambda *s: _rng.normal(s) * 0.05)(D, Hq * Dh) * D ** (-0.5)), 'wo': _w((lambda *s: _rng.normal(s) * 0.05)(Hq * Dh, D) * (Hq * Dh) ** (-0.5))}
    _A_in = _A_setup()

    def _B_setup():
        B, S, D, F, C = (4, 1, 512, 1376, 1)
        return {'x': _w((lambda *s: _rng.normal(s) * 0.05)(B, S, D)), 'w_r': _w((lambda *s: _rng.normal(s) * 0.05)(D)), 'w_gate': _w((lambda *s: _rng.normal(s) * 0.05)(D, F)), 'w_up': _w((lambda *s: _rng.normal(s) * 0.05)(D, F)), 'w_down': _w((lambda *s: _rng.normal(s) * 0.05)(F, D))}
    _B_in = _B_setup()
    return {'A_x': _A_in['x'], 'A_k_cache': _A_in['k_cache'], 'A_v_cache': _A_in['v_cache'], 'A_wq': _A_in['wq'], 'A_wo': _A_in['wo'], 'B_x': _B_in['x'], 'B_w_r': _B_in['w_r'], 'B_w_gate': _B_in['w_gate'], 'B_w_up': _B_in['w_up'], 'B_w_down': _B_in['w_down'], 'c': _w((lambda *s: _rng.normal(s) * 0.05)(4, 512)), 'w_mod': _w((lambda *s: _rng.normal(s) * 0.05)(512, 6 * 512) * 512 ** (-0.5))}

def reference(A_x, A_k_cache, A_v_cache, A_wq, A_wo, B_x, B_w_r, B_w_gate, B_w_up, B_w_down, c, w_mod):

    def _A_ref(x, k_cache, v_cache, wq, wo):
        B, Sq, D = x.shape
        Hq, Dh = (32, 128)
        Hkv = k_cache.shape[1]
        rep = Hq // Hkv
        q = (lambda x, *d: x.transpose(*d))((x @ wq).reshape(B, Sq, Hq, Dh), 0, 2, 1, 3)
        k = jnp.repeat(k_cache, rep, axis=1)
        v = jnp.repeat(v_cache, rep, axis=1)
        scores = jnp.einsum('bhqd,bhkd->bhqk', q, k) * Dh ** (-0.5)
        p = _softmax(scores, axis=-1)
        o = jnp.einsum('bhqk,bhkd->bhqd', p, v)
        return (lambda x, *d: x.transpose(*d))(o, 0, 2, 1, 3).reshape(B, Sq, Hq * Dh) @ wo

    def _B_ref(x, w_r, w_gate, w_up, w_down):
        B, S, D = x.shape
        C = 1
        r = x @ w_r
        idx = jnp.argsort(-r, axis=-1)[:, :C]
        idx_e = jnp.repeat(idx.reshape(B, C, 1), D, axis=2)
        x_sel = jnp.take_along_axis(x, idx_e, axis=1)
        g = _silu(x_sel @ w_gate)
        u = x_sel @ w_up
        y = g * u @ w_down
        r_sel = _sigmoid(jnp.take_along_axis(r, idx, axis=1))
        y = y * r_sel.reshape(B, C, 1)
        b_off = (jnp.arange(B) * S).reshape(B, 1)
        flat_idx = (idx + b_off).reshape(B * C)
        zero = (x * 0.0).reshape(B * S, D)
        upd = _scatter_add(zero, flat_idx, y.reshape(B * C, D), axis=0)
        return x + upd.reshape(B, S, D)
    x = A_x
    mod = (_silu(c) @ w_mod).reshape(c.shape[0], 6, 1, -1)
    sa, ca, ga, sb, cb, gb = (mod[:, 0].copy(), mod[:, 1].copy(), mod[:, 2].copy(), mod[:, 3].copy(), mod[:, 4].copy(), mod[:, 5].copy())
    h = _layernorm(x, axis=-1) * (1 + ca) + sa
    x = x + ga * _A_ref(h, A_k_cache, A_v_cache, A_wq, A_wo)
    h = _layernorm(x, axis=-1) * (1 + cb) + sb
    x = x + gb * _B_ref(h, B_w_r, B_w_gate, B_w_up, B_w_down)
    return x
```

```python
import functools
import jax
import jax.numpy as jnp
import numpy as np
from jax import lax
from jax.experimental import pallas as pl
from jax.experimental.pallas import tpu as pltpu

B, D, H, SK, DH, F = 4, 512, 32, 8192, 128, 1376
LOG2E = 1.4426950408889634


def _make_kernel(T=1024, ROWS=128, NBUF=3, wchunk=True, skew=0, hskew=0, wd_split=(1376,), nobc=False):
    NCH = SK // T
    NT = T // ROWS
    NITER = H * NCH
    f32, bf16 = jnp.float32, jnp.bfloat16

    def kernel(x_hbm, c_hbm, wr_hbm, k_hbm, v_hbm, wq_hbm, wo_hbm, wmod_hbm, wgt_hbm, wut_hbm, wd_hbm,
               o_hbm,
               kbuf, vbuf, x_s, c_s, wr_s, wq_s, wo_s, wmod_s, wg_s, wu_s, wd_s, q_s, o_s, kv_sem, w_sem):

        def issue(i, slot):
            h = i // NCH
            c = i % NCH
            for t in range(NT):
                for b in range(B):
                    cb_ = (c + b * skew) % NCH if skew else c
                    hb_ = (h + b * hskew) % H if hskew else h
                    src_rows = pl.ds(pl.multiple_of(cb_ * T + t * ROWS, ROWS), ROWS)
                    pltpu.make_async_copy(k_hbm.at[b, hb_, src_rows, :], kbuf.at[slot, b, pl.ds(t * ROWS, ROWS), :],
                                          kv_sem.at[slot, 0]).start(priority=0)
                    pltpu.make_async_copy(v_hbm.at[b, hb_, src_rows, :], vbuf.at[slot, b, pl.ds(t * ROWS, ROWS), :],
                                          kv_sem.at[slot, 1]).start(priority=1)

        def wait_k(slot):
            pltpu.make_async_copy(kbuf.at[slot], kbuf.at[slot], kv_sem.at[slot, 0]).wait()

        def wait_v(slot):
            pltpu.make_async_copy(vbuf.at[slot], vbuf.at[slot], kv_sem.at[slot, 1]).wait()

        def start_w(src, dst, sem, r0, nrows, c0, ncols):
            if not wchunk:
                pltpu.make_async_copy(src.at[pl.ds(r0, nrows), pl.ds(c0, ncols)], dst.at[pl.ds(r0, nrows), pl.ds(c0, ncols)], sem).start()
                return
            pc = min(ncols, 1024)
            pr = 16 * 1024 // pc
            ncj = ncols // pc
            nri = nrows // pr
            assert nri * pr == nrows and ncj * pc == ncols
            n = nri * ncj
            def one(idx, prio):
                ri = idx // ncj
                cj = idx % ncj
                rs = pl.ds(pl.multiple_of(r0 + ri * pr, 16), pr)
                cs = pl.ds(pl.multiple_of(c0 + cj * pc, 128), pc)
                pltpu.make_async_copy(src.at[rs, cs], dst.at[rs, cs], sem).start(priority=prio)
            def body(j, _):
                one(2 * j, 0)
                one(2 * j + 1, 1)
                return _
            lax.fori_loop(0, n // 2, body, 0)
            if n % 2:
                one(n - 1, 0)

        def wait_w(dst, sem, r0, nrows, c0, ncols):
            v = dst.at[pl.ds(r0, nrows), pl.ds(c0, ncols)]
            pltpu.make_async_copy(v, v, sem).wait()

        small = [pltpu.make_async_copy(x_hbm, x_s, w_sem.at[0]),
                 pltpu.make_async_copy(c_hbm, c_s, w_sem.at[1]),
                 pltpu.make_async_copy(wr_hbm, wr_s, w_sem.at[2])]
        small[1].start()
        small[0].start()
        start_w(wmod_hbm, wmod_s, w_sem.at[3], 0, D, 0, 2 * D)
        start_w(wq_hbm, wq_s, w_sem.at[4], 0, D, 0, H * DH)
        for s in range(NBUF):
            issue(s, s)
        start_w(wo_hbm, wo_s, w_sem.at[5], 0, H * DH, 0, D)
        start_w(wmod_hbm, wmod_s, w_sem.at[6], 0, D, 2 * D, 4 * D)
        small[2].start()

        small[1].wait()
        cc = c_s[...].astype(f32)
        sc = (cc * jax.nn.sigmoid(cc)).astype(bf16)
        small[0].wait()
        x = x_s[...].astype(f32)

        def ln(v):
            m = jnp.mean(v, axis=-1, keepdims=True)
            d = v - m
            var = jnp.mean(d * d, axis=-1, keepdims=True)
            return d * lax.rsqrt(var + 1e-5)

        xn = ln(x)
        wait_w(wmod_s, w_sem.at[3], 0, D, 0, 2 * D)
        mod_a = jnp.dot(sc, wmod_s[:, 0:2 * D], preferred_element_type=f32)
        sa, ca = mod_a[:, 0:D], mod_a[:, D:2 * D]
        h1 = xn * (1.0 + ca) + sa
        wait_w(wq_s, w_sem.at[4], 0, D, 0, H * DH)
        q = jnp.dot(h1.astype(bf16), wq_s[...], preferred_element_type=f32)
        q_s[...] = q.astype(bf16)

        scale = (DH ** -0.5) * LOG2E
        row_t = lax.broadcasted_iota(jnp.int32, (B, T), 0)
        row_d = lax.broadcasted_iota(jnp.int32, (B, DH), 0)

        def head_body(h, attn):
            if hskew:
                qh = None
                for b in range(B):
                    hb_ = (h + b * hskew) % H
                    qb_ = q_s[:, pl.ds(pl.multiple_of(hb_ * DH, DH), DH)]
                    qh = qb_ if b == 0 else jnp.where(row_d == b, qb_, qh)
            else:
                qh = q_s[:, pl.ds(pl.multiple_of(h * DH, DH), DH)]

            def chunk_body(c, carry):
                m, l, acc = carry
                i = h * NCH + c
                slot = i % NBUF
                wait_k(slot)
                s = None
                for b in range(B):
                    sb_ = lax.dot_general(qh, kbuf[slot, b], (((1,), (1,)), ((), ())), preferred_element_type=f32)
                    s = sb_ if b == 0 else jnp.where(row_t == b, sb_, s)
                s = s * scale
                m_new = jnp.maximum(m, jnp.max(s, axis=1, keepdims=True))
                alpha = jnp.exp2(m - m_new)
                p = jnp.exp2(s - m_new)
                l = l * alpha + jnp.sum(p, axis=1, keepdims=True)
                pb = p.astype(bf16)
                wait_v(slot)
                o = None
                for b in range(B):
                    ob = jnp.dot(pb, vbuf[slot, b], preferred_element_type=f32)
                    o = ob if b == 0 else jnp.where(row_d == b, ob, o)
                acc = acc * alpha + o

                @pl.when(i + NBUF < NITER)
                def _():
                    issue(i + NBUF, slot)

                @pl.when(i + NBUF == NITER)
                def _():
                    start_w(wgt_hbm, wg_s, w_sem.at[7], 0, F, 0, D)
                    start_w(wut_hbm, wu_s, w_sem.at[8], 0, F, 0, D)
                    r0 = 0
                    for j, nr in enumerate(wd_split):
                        start_w(wd_hbm, wd_s, w_sem.at[9 + j], r0, nr, 0, D)
                        r0 += nr
                return m_new, l, acc

            m0 = jnp.full((B, 1), -jnp.inf, f32)
            l0 = jnp.zeros((B, 1), f32)
            a0 = jnp.zeros((B, DH), f32)
            m, l, acc = lax.fori_loop(0, NCH, chunk_body, (m0, l0, a0))
            oh = (acc / l).astype(bf16)

            @pl.when(h == 0)
            def _():
                wait_w(wo_s, w_sem.at[5], 0, H * DH, 0, D)
            if hskew:
                for b in range(B):
                    hb_ = (h + b * hskew) % H
                    ob = jnp.dot(oh, wo_s[pl.ds(pl.multiple_of(hb_ * DH, DH), DH), :], preferred_element_type=f32)
                    attn = attn + jnp.where(lax.broadcasted_iota(jnp.int32, (B, D), 0) == b, ob, 0.0)
            else:
                attn = attn + jnp.dot(oh, wo_s[pl.ds(pl.multiple_of(h * DH, DH), DH), :], preferred_element_type=f32)
            return attn

        attn = lax.fori_loop(0, H, head_body, jnp.zeros((B, D), f32))

        wait_w(wmod_s, w_sem.at[6], 0, D, 2 * D, 4 * D)
        mod_b = jnp.dot(sc, wmod_s[:, 2 * D:6 * D], preferred_element_type=f32)
        ga, sb, cb, gb = [mod_b[:, j * D:(j + 1) * D] for j in range(4)]
        x1 = x + ga * attn
        h2 = ln(x1) * (1.0 + cb) + sb
        h2b = h2.astype(bf16)
        small[2].wait()
        wr = wr_s[...].reshape(1, D).astype(f32)
        r = jnp.sum(h2b.astype(f32) * wr, axis=-1, keepdims=True)
        nt = (((1,), (1,)), ((), ()))
        wait_w(wg_s, w_sem.at[7], 0, F, 0, D)
        g = lax.dot_general(h2b, wg_s[...], nt, preferred_element_type=f32)
        wait_w(wu_s, w_sem.at[8], 0, F, 0, D)
        u = lax.dot_general(h2b, wu_s[...], nt, preferred_element_type=f32)
        a = ((g * jax.nn.sigmoid(g)) * u).astype(bf16)
        y = None
        r0 = 0
        for j, nr in enumerate(wd_split):
            wait_w(wd_s, w_sem.at[9 + j], r0, nr, 0, D)
            yj = jnp.dot(a[:, r0:r0 + nr], wd_s[r0:r0 + nr, :], preferred_element_type=f32)
            y = yj if y is None else y + yj
            r0 += nr
        y = y * jax.nn.sigmoid(r)
        upd = h2 * 0.0 + y
        out = x1 + gb * (h2 + upd)
        o_s[...] = out.astype(o_s.dtype)
        cp = pltpu.make_async_copy(o_s, o_hbm, w_sem.at[0])
        cp.start()
        cp.wait()

    @jax.jit
    def fn(A_x, A_k_cache, A_v_cache, A_wq, A_wo, B_x, B_w_r, B_w_gate, B_w_up, B_w_down, c, w_mod):
        hbm = pl.BlockSpec(memory_space=pltpu.HBM)
        out = pl.pallas_call(
            kernel,
            out_shape=jax.ShapeDtypeStruct((B, D), A_x.dtype),
            in_specs=[hbm] * 11,
            out_specs=hbm,
            scratch_shapes=[
                pltpu.VMEM((NBUF, B, T, DH), bf16), pltpu.VMEM((NBUF, B, T, DH), bf16),
                pltpu.VMEM((B, D), bf16), pltpu.VMEM((B, D), bf16), pltpu.VMEM((D,), bf16),
                pltpu.VMEM((D, H * DH), bf16), pltpu.VMEM((H * DH, D), bf16), pltpu.VMEM((D, 6 * D), bf16),
                pltpu.VMEM((F, D), bf16), pltpu.VMEM((F, D), bf16), pltpu.VMEM((F, D), bf16),
                pltpu.VMEM((B, H * DH), bf16), pltpu.VMEM((B, D), bf16),
                pltpu.SemaphoreType.DMA((NBUF, 2)), pltpu.SemaphoreType.DMA((9 + len(wd_split),)),
            ],
            compiler_params=pltpu.CompilerParams(vmem_limit_bytes=100 * 1024 * 1024, disable_bounds_checks=nobc),
        )(A_x.reshape(B, D), c, B_w_r, A_k_cache, A_v_cache, A_wq, A_wo, w_mod, B_w_gate.T, B_w_up.T, B_w_down)
        return out.reshape(B, 1, D)
    return fn


_IMPL = _make_kernel()


@jax.jit
def pallas_adaLN_cond__gqa_block_cached__moe_arch_mod__decode_kernel(
    A_x, A_k_cache, A_v_cache, A_wq, A_wo, B_x, B_w_r, B_w_gate, B_w_up, B_w_down, c, w_mod
):
    return _IMPL(A_x, A_k_cache, A_v_cache, A_wq, A_wo, B_x, B_w_r, B_w_gate, B_w_up, B_w_down, c, w_mod)
```

```python
import jax
import jax.numpy as jnp
import numpy as np
from jax import lax
from jax.experimental import pallas as pl
from jax.experimental.pallas import tpu as pltpu

B, D, H, SK, DH, F = 4, 512, 32, 8192, 128, 1376
LOG2E = 1.4426950408889634


def _rotate(pieces, ns):
    n = len(pieces)
    seg = -(-n // ns)
    return [pieces[s * seg + i] for i in range(seg) for s in range(ns) if s * seg + i < n]


def _interleave(a, b):
    out = []
    for i in range(max(len(a), len(b))):
        out += a[i:i + 1] + b[i:i + 1]
    return out


def make_kernel(T=1024, NBUF=3, vrow=64, krow=0, ns=8, ffn_mode=0, early_mode=0, xp=0, q16=False, vl=64, xfirst=False, wrpos=0, loop_early=True, loop_ffn=False, dsplit=0, slotloop=False, nosem=False, nobc=True):
    ROWS = 128
    NCH = SK // T
    NT = T // ROWS
    NITER = H * NCH
    f32, bf16 = jnp.float32, jnp.bfloat16

    kv_pieces = []
    for a, sh in ((0, krow), (1, vrow)):
        if sh:
            kv_pieces += [(a, b, 0, sh) for b in range(B)]
    for t in range(NT):
        for a, sh in ((0, krow), (1, vrow)):
            nr = ROWS if (t < NT - 1 or sh == 0) else ROWS - sh
            kv_pieces += [(a, b, sh + t * ROWS, nr) for b in range(B)]

    mod_a = _rotate([('moda', r, 16, 0, 1024) for r in range(0, D, 16)], ns)
    mod_b = _rotate([('modb', r, 8, 1024, 2048) for r in range(0, D, 8)], ns)
    w_q = _rotate([('q', r, 8, c, 2048) for r in range(0, D, 8) for c in (0, 2048)], ns)
    if q16:
        w_q = _rotate([('q', r, 16, c, 1024) for r in range(0, D, 16) for c in (0, 1024, 2048, 3072)], ns)
    w_o = _rotate([('o', r, 32, 0, D) for r in range(0, H * DH, 32)], ns)
    if ffn_mode == 0:
        w_g = _rotate([('g', r, 32, 0, D) for r in range(0, F, 32)], ns)
        w_u = _rotate([('u', r, 32, 0, D) for r in range(0, F, 32)], ns)
        w_d = _rotate([('d', r, 32, 0, D) for r in range(0, F, 32)], ns)
        if dsplit:
            w_d = _rotate([('d', r, 32, 0, D) for r in range(0, dsplit, 32)], ns) + _rotate([('d2', r, 32, 0, D) for r in range(dsplit, F, 32)], ns)
        ffn = w_g + w_u + w_d
    else:
        w_g = _rotate([('g', r, 32, 0, D) for r in range(0, F, 32)], ns // 2)
        w_u = _rotate([('u', r, 32, 0, D) for r in range(0, F, 32)], ns // 2)
        w_d = _rotate([('d', r, 32, 0, D) for r in range(0, F, 32)], ns)
        ffn = _interleave(w_g, w_u) + w_d

    def kernel(x_hbm, c_hbm, wr_hbm, k_hbm, v_hbm, wq_hbm, wo_hbm, wmod_hbm, wgt_hbm, wut_hbm, wd_hbm,
               o_hbm,
               kbuf, vbuf, x_s, c_s, wr_s, wq_s, wo_s, wmod_s, wg_s, wu_s, wd_s, q_s, o_s, kv_sem, w_sem):
        wrefs = {
            'moda': (wmod_hbm, wmod_s, 3), 'modb': (wmod_hbm, wmod_s, 6), 'q': (wq_hbm, wq_s, 4),
            'o': (wo_hbm, wo_s, 5), 'g': (wgt_hbm, wg_s, 7), 'u': (wut_hbm, wu_s, 8), 'd': (wd_hbm, wd_s, 9), 'd2': (wd_hbm, wd_s, 10),
        }

        def start_weights(pieces):
            for n, (name, r0, nr, c0, nc) in enumerate(pieces):
                src, dst, s = wrefs[name]
                pltpu.make_async_copy(src.at[pl.ds(r0, nr), pl.ds(c0, nc)], dst.at[pl.ds(r0, nr), pl.ds(c0, nc)],
                                      w_sem.at[s]).start(priority=n % 2)

        def start_loop(name, r0, nrows, c0, ncols, pr, pc, nsr):
            src, dst, s_ = wrefs[name]
            ncj = ncols // pc
            nri = nrows // pr
            n = nri * ncj
            seg = -(-n // nsr)
            def one(idx, prio):
                ri = idx // ncj
                cj = idx % ncj
                rs = pl.ds(pl.multiple_of(r0 + ri * pr, 8), pr)
                cs = pl.ds(pl.multiple_of(c0 + cj * pc, 128), pc)
                pltpu.make_async_copy(src.at[rs, cs], dst.at[rs, cs], w_sem.at[s_]).start(priority=prio)
            if n % nsr == 0 and nsr % 2 == 0:
                def body(j, _):
                    for u in range(nsr):
                        one(u * seg + j, u % 2)
                    return _
                lax.fori_loop(0, seg, body, 0)
            else:
                def body(j, _):
                    one(2 * j, 0)
                    one(2 * j + 1, 1)
                    return _
                lax.fori_loop(0, n // 2, body, 0)
                if n % 2:
                    one(n - 1, 0)

        def wait_weights(name, c0=0, nc=None):
            _, dst, s = wrefs[name]
            v = dst if nc is None else dst.at[:, pl.ds(c0, nc)]
            pltpu.make_async_copy(v, v, w_sem.at[s]).wait()

        def issue(i, slot):
            h = i // NCH
            row0 = (i % NCH) * T
            for n, (a, b, r0, nr) in enumerate(kv_pieces):
                src, dst = ((k_hbm, kbuf), (v_hbm, vbuf))[a]
                pltpu.make_async_copy(src.at[b, h, pl.ds(pl.multiple_of(row0 + r0, 16), nr), :],
                                      dst.at[slot, b, pl.ds(r0, nr), :],
                                      kv_sem.at[slot, a]).start(priority=n % 2)

        def wait_kv(buf, slot, a):
            pltpu.make_async_copy(buf.at[slot], buf.at[slot], kv_sem.at[slot, a]).wait()

        x_cp = pltpu.make_async_copy(x_hbm, x_s, w_sem.at[0])
        c_cp = pltpu.make_async_copy(c_hbm, c_s, w_sem.at[1])
        wr_cp = pltpu.make_async_copy(wr_hbm, wr_s, w_sem.at[2])
        c_cp.start()
        x_cp.start(priority=xp)
        if loop_early:
            start_loop('moda', 0, D, 0, 1024, 16, 1024, ns)
            start_loop('q', 0, D, 0, 4096, 16, 1024, ns)
        else:
            start_weights(mod_a)
            start_weights(w_q)
        if slotloop:
            def _first(s, carry):
                issue(s, s)
                return carry
            lax.fori_loop(0, NBUF, _first, 0)
        else:
            for s in range(NBUF):
                issue(s, s)
        if loop_early:
            start_loop('o', 0, H * DH, 0, D, 32, D, ns)
            start_loop('modb', 0, D, 1024, 2048, 8, 2048, ns)
        else:
            start_weights(_interleave(w_o, mod_b) if early_mode == 0 else w_o + mod_b)
        wr_cp.start()

        def ln(v):
            m = jnp.mean(v, axis=-1, keepdims=True)
            d = v - m
            var = jnp.mean(d * d, axis=-1, keepdims=True)
            return d * lax.rsqrt(var + 1e-5)

        c_cp.wait()
        cc = c_s[...].astype(f32)
        sc = (cc * jax.nn.sigmoid(cc)).astype(bf16)
        x_cp.wait()
        x = x_s[...].astype(f32)
        xn = ln(x)
        wait_weights('moda', 0, 2 * D)
        mod_a_v = jnp.dot(sc, wmod_s[:, 0:2 * D], preferred_element_type=f32)
        h1 = xn * (1.0 + mod_a_v[:, D:2 * D]) + mod_a_v[:, 0:D]
        wait_weights('q')
        q_s[...] = jnp.dot(h1.astype(bf16), wq_s[...], preferred_element_type=f32).astype(bf16)

        scale = (DH ** -0.5) * LOG2E
        row_t = lax.broadcasted_iota(jnp.int32, (B, T), 0)
        row_d = lax.broadcasted_iota(jnp.int32, (B, DH), 0)
        nt_dims = (((1,), (1,)), ((), ()))

        def head_body(h, attn):
            qh = q_s[:, pl.ds(pl.multiple_of(h * DH, DH), DH)]

            def chunk_body(c, carry):
                m, l, acc = carry
                i = h * NCH + c
                slot = i % NBUF
                wait_kv(kbuf, slot, 0)
                s = None
                for b in range(B):
                    s_b = lax.dot_general(qh, kbuf[slot, b], nt_dims, preferred_element_type=f32)
                    s = s_b if b == 0 else jnp.where(row_t == b, s_b, s)
                s = s * scale
                m_new = jnp.maximum(m, jnp.max(s, axis=1, keepdims=True))
                alpha = jnp.exp2(m - m_new)
                p = jnp.exp2(s - m_new)
                l = l * alpha + jnp.sum(p, axis=1, keepdims=True)
                pb = p.astype(bf16)
                wait_kv(vbuf, slot, 1)
                o = None
                for b in range(B):
                    o_b = jnp.dot(pb, vbuf[slot, b], preferred_element_type=f32)
                    o = o_b if b == 0 else jnp.where(row_d == b, o_b, o)
                acc = acc * alpha + o

                @pl.when(i + NBUF < NITER)
                def _():
                    issue(i + NBUF, slot)

                @pl.when(i + NBUF == NITER)
                def _():
                    if loop_ffn:
                        for nm in 'gud':
                            start_loop(nm, 0, F, 0, D, 32, D, 1)
                    else:
                        start_weights(ffn)
                return m_new, l, acc

            init = (jnp.full((B, 1), -jnp.inf, f32), jnp.zeros((B, 1), f32), jnp.zeros((B, DH), f32))
            _, l, acc = lax.fori_loop(0, NCH, chunk_body, init)
            oh = (acc / l).astype(bf16)

            @pl.when(h == 0)
            def _():
                wait_weights('o')
            return attn + jnp.dot(oh, wo_s[pl.ds(pl.multiple_of(h * DH, DH), DH), :], preferred_element_type=f32)

        attn = lax.fori_loop(0, H, head_body, jnp.zeros((B, D), f32))

        wait_weights('modb', 2 * D, 4 * D)
        mod_b_v = jnp.dot(sc, wmod_s[:, 2 * D:6 * D], preferred_element_type=f32)
        ga, sb, cb, gb = [mod_b_v[:, j * D:(j + 1) * D] for j in range(4)]
        x1 = x + ga * attn
        h2 = ln(x1) * (1.0 + cb) + sb
        h2b = h2.astype(bf16)
        wr_cp.wait()
        r = jnp.sum(h2b.astype(f32) * wr_s[...].reshape(1, D).astype(f32), axis=-1, keepdims=True)
        wait_weights('g')
        g = lax.dot_general(h2b, wg_s[...], nt_dims, preferred_element_type=f32)
        wait_weights('u')
        u = lax.dot_general(h2b, wu_s[...], nt_dims, preferred_element_type=f32)
        a = ((g * jax.nn.sigmoid(g)) * u).astype(bf16)
        if dsplit:
            v1 = wd_s.at[pl.ds(0, dsplit), :]
            pltpu.make_async_copy(v1, v1, w_sem.at[9]).wait()
            y = jnp.dot(a[:, :dsplit], wd_s[0:dsplit, :], preferred_element_type=f32)
            v2 = wd_s.at[pl.ds(dsplit, F - dsplit), :]
            pltpu.make_async_copy(v2, v2, w_sem.at[10]).wait()
            y = (y + jnp.dot(a[:, dsplit:], wd_s[dsplit:F, :], preferred_element_type=f32)) * jax.nn.sigmoid(r)
        else:
            wait_weights('d')
            y = jnp.dot(a, wd_s[...], preferred_element_type=f32) * jax.nn.sigmoid(r)
        out = x1 + gb * (h2 + (h2 * 0.0 + y))
        o_s[...] = out.astype(o_s.dtype)
        o_cp = pltpu.make_async_copy(o_s, o_hbm, w_sem.at[0])
        o_cp.start()
        o_cp.wait()

    @jax.jit
    def fn(A_x, A_k_cache, A_v_cache, A_wq, A_wo, B_x, B_w_r, B_w_gate, B_w_up, B_w_down, c, w_mod):
        hbm = pl.BlockSpec(memory_space=pltpu.HBM)
        out = pl.pallas_call(
            kernel,
            out_shape=jax.ShapeDtypeStruct((B, D), A_x.dtype),
            in_specs=[hbm] * 11,
            out_specs=hbm,
            scratch_shapes=[
                pltpu.VMEM((NBUF, B, T, DH), bf16), pltpu.VMEM((NBUF, B, T, DH), bf16),
                pltpu.VMEM((B, D), bf16), pltpu.VMEM((B, D), bf16), pltpu.VMEM((D,), bf16),
                pltpu.VMEM((D, H * DH), bf16), pltpu.VMEM((H * DH, D), bf16), pltpu.VMEM((D, 6 * D), bf16),
                pltpu.VMEM((F, D), bf16), pltpu.VMEM((F, D), bf16), pltpu.VMEM((F, D), bf16),
                pltpu.VMEM((B, H * DH), bf16), pltpu.VMEM((B, D), bf16),
                pltpu.SemaphoreType.DMA((NBUF, 2)), pltpu.SemaphoreType.DMA((11,)),
            ],
            compiler_params=pltpu.CompilerParams(vmem_limit_bytes=vl * 1024 * 1024, disable_bounds_checks=nobc, disable_semaphore_checks=nosem),
        )(A_x.reshape(B, D), c, B_w_r, A_k_cache, A_v_cache, A_wq, A_wo, w_mod, B_w_gate.T, B_w_up.T, B_w_down)
        return out.reshape(B, 1, D)
    return fn


_IMPL = make_kernel(T=1024, NBUF=3, slotloop=True)


@jax.jit
def pallas_adaLN_cond__gqa_block_cached__moe_arch_mod__decode_kernel(
    A_x, A_k_cache, A_v_cache, A_wq, A_wo, B_x, B_w_r, B_w_gate, B_w_up, B_w_down, c, w_mod
):
    return _IMPL(A_x, A_k_cache, A_v_cache, A_wq, A_wo, B_x, B_w_r, B_w_gate, B_w_up, B_w_down, c, w_mod)
```

```python
import jax
import jax.numpy as jnp
from jax import lax
from jax.experimental import pallas as pl
from jax.experimental.pallas import tpu as pltpu

B, D, H, SK, DH, F = 4, 512, 32, 8192, 128, 1376

T = 2048
NBUF = 2
ROWS = 128
V_SHIFT = 64
NSTREAM = 8
NCH = SK // T
NITER = H * NCH

LOG2E = 1.4426950408889634
NT_DIMS = (((1,), (1,)), ((), ()))

S_X, S_C, S_WR, S_MODA, S_Q, S_O, S_MODB, S_G, S_U, S_D = range(10)


def _kv_pieces():
    pieces = [(1, b, 0, V_SHIFT) for b in range(B)]
    for t in range(T // ROWS):
        pieces += [(0, b, t * ROWS, ROWS) for b in range(B)]
        v_rows = ROWS if (t + 1) * ROWS < T else ROWS - V_SHIFT
        pieces += [(1, b, V_SHIFT + t * ROWS, v_rows) for b in range(B)]
    return pieces


def _rotated_rows(nrows, step):
    n = nrows // step
    seg = -(-n // NSTREAM)
    return [(s * seg + i) * step for i in range(seg) for s in range(NSTREAM) if s * seg + i < n]


def _layernorm(v):
    mean = jnp.mean(v, axis=-1, keepdims=True)
    d = v - mean
    var = jnp.mean(d * d, axis=-1, keepdims=True)
    return d * lax.rsqrt(var + 1e-5)


def _kernel(x_hbm, c_hbm, wr_hbm, k_hbm, v_hbm, wq_hbm, wo_hbm, wmod_hbm, wgt_hbm, wut_hbm, wd_hbm,
            o_hbm,
            kbuf, vbuf, x_s, c_s, wr_s, wq_s, wo_s, wmod_s, wg_s, wu_s, wd_s, q_s, o_s, kv_sem, w_sem):
    f32, bf16 = jnp.float32, jnp.bfloat16

    def start_tiles(src, dst, sem, col0, ncols, pr, pc):
        ncj = ncols // pc
        seg = (src.shape[0] // pr) * ncj // NSTREAM

        def body(j, carry):
            for u in range(NSTREAM):
                idx = u * seg + j
                rows = pl.ds(pl.multiple_of((idx // ncj) * pr, 8), pr)
                cols = pl.ds(pl.multiple_of(col0 + (idx % ncj) * pc, 128), pc)
                pltpu.make_async_copy(src.at[rows, cols], dst.at[rows, cols], sem).start(priority=u % 2)
            return carry
        lax.fori_loop(0, seg, body, 0)

    def start_ffn_weights():
        n = 0
        for src, dst, s in ((wgt_hbm, wg_s, S_G), (wut_hbm, wu_s, S_U), (wd_hbm, wd_s, S_D)):
            for r in _rotated_rows(F, 32):
                pltpu.make_async_copy(src.at[pl.ds(r, 32)], dst.at[pl.ds(r, 32)],
                                      w_sem.at[s]).start(priority=n % 2)
                n += 1

    def wait_all(view, s):
        pltpu.make_async_copy(view, view, w_sem.at[s]).wait()

    def start_slot(i, slot):
        h = i // NCH
        row0 = (i % NCH) * T
        for n, (a, b, r0, nr) in enumerate(_kv_pieces()):
            src, dst = ((k_hbm, kbuf), (v_hbm, vbuf))[a]
            pltpu.make_async_copy(src.at[b, h, pl.ds(pl.multiple_of(row0 + r0, 16), nr), :],
                                  dst.at[slot, b, pl.ds(r0, nr), :],
                                  kv_sem.at[slot, a]).start(priority=n % 2)

    def wait_slot(buf, slot, a):
        pltpu.make_async_copy(buf.at[slot], buf.at[slot], kv_sem.at[slot, a]).wait()

    x_cp = pltpu.make_async_copy(x_hbm, x_s, w_sem.at[S_X])
    c_cp = pltpu.make_async_copy(c_hbm, c_s, w_sem.at[S_C])
    wr_cp = pltpu.make_async_copy(wr_hbm, wr_s, w_sem.at[S_WR])
    c_cp.start()
    x_cp.start()
    start_tiles(wmod_hbm, wmod_s, w_sem.at[S_MODA], 0, 2 * D, 16, 1024)
    start_tiles(wq_hbm, wq_s, w_sem.at[S_Q], 0, H * DH, 16, 1024)

    def first_slots(s, carry):
        start_slot(s, s)
        return carry
    lax.fori_loop(0, NBUF, first_slots, 0)
    start_tiles(wo_hbm, wo_s, w_sem.at[S_O], 0, D, 32, D)
    start_tiles(wmod_hbm, wmod_s, w_sem.at[S_MODB], 2 * D, 4 * D, 8, 2048)
    wr_cp.start()

    c_cp.wait()
    cc = c_s[...].astype(f32)
    sc = (cc * jax.nn.sigmoid(cc)).astype(bf16)
    x_cp.wait()
    x = x_s[...].astype(f32)
    xn = _layernorm(x)
    wait_all(wmod_s.at[:, pl.ds(0, 2 * D)], S_MODA)
    mod_a = jnp.dot(sc, wmod_s[:, 0:2 * D], preferred_element_type=f32)
    h1 = xn * (1.0 + mod_a[:, D:2 * D]) + mod_a[:, 0:D]
    wait_all(wq_s, S_Q)
    q_s[...] = jnp.dot(h1.astype(bf16), wq_s[...], preferred_element_type=f32).astype(bf16)

    scale = (DH ** -0.5) * LOG2E
    row_t = lax.broadcasted_iota(jnp.int32, (B, T), 0)
    row_d = lax.broadcasted_iota(jnp.int32, (B, DH), 0)

    def head_body(h, attn):
        qh = q_s[:, pl.ds(pl.multiple_of(h * DH, DH), DH)]

        def chunk_body(c, carry):
            m, l, acc = carry
            i = h * NCH + c
            slot = i % NBUF
            wait_slot(kbuf, slot, 0)
            s = lax.dot_general(qh, kbuf[slot, 0], NT_DIMS, preferred_element_type=f32)
            for b in range(1, B):
                s_b = lax.dot_general(qh, kbuf[slot, b], NT_DIMS, preferred_element_type=f32)
                s = jnp.where(row_t == b, s_b, s)
            s = s * scale
            m_new = jnp.maximum(m, jnp.max(s, axis=1, keepdims=True))
            alpha = jnp.exp2(m - m_new)
            p = jnp.exp2(s - m_new)
            l = l * alpha + jnp.sum(p, axis=1, keepdims=True)
            pb = p.astype(bf16)
            wait_slot(vbuf, slot, 1)
            o = jnp.dot(pb, vbuf[slot, 0], preferred_element_type=f32)
            for b in range(1, B):
                o_b = jnp.dot(pb, vbuf[slot, b], preferred_element_type=f32)
                o = jnp.where(row_d == b, o_b, o)
            acc = acc * alpha + o

            @pl.when(i + NBUF < NITER)
            def _():
                start_slot(i + NBUF, slot)

            @pl.when(i + NBUF == NITER)
            def _():
                start_ffn_weights()
            return m_new, l, acc

        init = (jnp.full((B, 1), -jnp.inf, f32), jnp.zeros((B, 1), f32), jnp.zeros((B, DH), f32))
        _, l, acc = lax.fori_loop(0, NCH, chunk_body, init)
        oh = (acc / l).astype(bf16)

        @pl.when(h == 0)
        def _():
            wait_all(wo_s, S_O)
        wo_h = wo_s[pl.ds(pl.multiple_of(h * DH, DH), DH), :]
        return attn + jnp.dot(oh, wo_h, preferred_element_type=f32)

    attn = lax.fori_loop(0, H, head_body, jnp.zeros((B, D), f32))

    wait_all(wmod_s.at[:, pl.ds(2 * D, 4 * D)], S_MODB)
    mod_b = jnp.dot(sc, wmod_s[:, 2 * D:6 * D], preferred_element_type=f32)
    ga, sb, cb, gb = [mod_b[:, j * D:(j + 1) * D] for j in range(4)]
    x1 = x + ga * attn
    h2 = _layernorm(x1) * (1.0 + cb) + sb
    h2b = h2.astype(bf16)
    wr_cp.wait()
    r = jnp.sum(h2b.astype(f32) * wr_s[...].reshape(1, D).astype(f32), axis=-1, keepdims=True)
    wait_all(wg_s, S_G)
    g = lax.dot_general(h2b, wg_s[...], NT_DIMS, preferred_element_type=f32)
    wait_all(wu_s, S_U)
    u = lax.dot_general(h2b, wu_s[...], NT_DIMS, preferred_element_type=f32)
    a = ((g * jax.nn.sigmoid(g)) * u).astype(bf16)
    wait_all(wd_s, S_D)
    y = jnp.dot(a, wd_s[...], preferred_element_type=f32) * jax.nn.sigmoid(r)
    out = x1 + gb * (h2 + (h2 * 0.0 + y))
    o_s[...] = out.astype(o_s.dtype)
    o_cp = pltpu.make_async_copy(o_s, o_hbm, w_sem.at[S_X])
    o_cp.start()
    o_cp.wait()


@jax.jit
def pallas_adaLN_cond__gqa_block_cached__moe_arch_mod__decode_kernel(
    A_x: jax.Array,
    A_k_cache: jax.Array,
    A_v_cache: jax.Array,
    A_wq: jax.Array,
    A_wo: jax.Array,
    B_x: jax.Array,
    B_w_r: jax.Array,
    B_w_gate: jax.Array,
    B_w_up: jax.Array,
    B_w_down: jax.Array,
    c: jax.Array,
    w_mod: jax.Array,
):
    del B_x
    bf16 = jnp.bfloat16
    hbm = pl.BlockSpec(memory_space=pltpu.HBM)
    out = pl.pallas_call(
        _kernel,
        out_shape=jax.ShapeDtypeStruct((B, D), A_x.dtype),
        in_specs=[hbm] * 11,
        out_specs=hbm,
        scratch_shapes=[
            pltpu.VMEM((NBUF, B, T, DH), bf16),
            pltpu.VMEM((NBUF, B, T, DH), bf16),
            pltpu.VMEM((B, D), bf16),
            pltpu.VMEM((B, D), bf16),
            pltpu.VMEM((D,), bf16),
            pltpu.VMEM((D, H * DH), bf16),
            pltpu.VMEM((H * DH, D), bf16),
            pltpu.VMEM((D, 6 * D), bf16),
            pltpu.VMEM((F, D), bf16),
            pltpu.VMEM((F, D), bf16),
            pltpu.VMEM((F, D), bf16),
            pltpu.VMEM((B, H * DH), bf16),
            pltpu.VMEM((B, D), bf16),
            pltpu.SemaphoreType.DMA((NBUF, 2)),
            pltpu.SemaphoreType.DMA((10,)),
        ],
        compiler_params=pltpu.CompilerParams(
            vmem_limit_bytes=48 * 1024 * 1024,
            disable_bounds_checks=True,
            disable_semaphore_checks=True,
        ),
    )(A_x.reshape(B, D), c, B_w_r, A_k_cache, A_v_cache, A_wq, A_wo, w_mod, B_w_gate.T, B_w_up.T, B_w_down)
    return out.reshape(B, 1, D)
```

```python
import jax
import jax.numpy as jnp
from jax import lax
from jax.experimental import pallas as pl
from jax.experimental.pallas import tpu as pltpu

B, D, H, SK, DH, F = 4, 512, 32, 8192, 128, 1376

T = 2048
NBUF = 2
ROWS = 128
V_SHIFT = 64
NSTREAM = 8
NCH = SK // T
NITER = H * NCH

LOG2E = 1.4426950408889634
NT_DIMS = (((1,), (1,)), ((), ()))

S_X, S_C, S_WR, S_MODA, S_Q, S_O, S_MODB, S_G, S_U, S_D = range(10)


def _kv_pieces():
    pieces = [(1, b, 0, V_SHIFT) for b in range(B)]
    for t in range(T // ROWS):
        pieces += [(0, b, t * ROWS, ROWS) for b in range(B)]
        v_rows = ROWS if (t + 1) * ROWS < T else ROWS - V_SHIFT
        pieces += [(1, b, V_SHIFT + t * ROWS, v_rows) for b in range(B)]
    return pieces


def _rotated_rows(nrows, step):
    n = nrows // step
    seg = -(-n // NSTREAM)
    return [(s * seg + i) * step for i in range(seg) for s in range(NSTREAM) if s * seg + i < n]


def _layernorm(v):
    mean = jnp.mean(v, axis=-1, keepdims=True)
    d = v - mean
    var = jnp.mean(d * d, axis=-1, keepdims=True)
    return d * lax.rsqrt(var + 1e-5)


def _kernel(x_hbm, c_hbm, wr_hbm, k_hbm, v_hbm, wq_hbm, wo_hbm, wmod_hbm, wgt_hbm, wut_hbm, wd_hbm,
            o_hbm,
            kbuf, vbuf, x_s, c_s, wr_s, wq_s, wo_s, wmod_s, wg_s, wu_s, wd_s, q_s, o_s, kv_sem, w_sem):
    f32, bf16 = jnp.float32, jnp.bfloat16

    def start_tiles(src, dst, sem, col0, ncols, pr, pc):
        ncj = ncols // pc
        seg = (src.shape[0] // pr) * ncj // NSTREAM

        def body(j, carry):
            for u in range(NSTREAM):
                idx = u * seg + j
                rows = pl.ds(pl.multiple_of((idx // ncj) * pr, 8), pr)
                cols = pl.ds(pl.multiple_of(col0 + (idx % ncj) * pc, 128), pc)
                pltpu.make_async_copy(src.at[rows, cols], dst.at[rows, cols], sem).start(priority=u % 2)
            return carry
        lax.fori_loop(0, seg, body, 0)

    def start_ffn_weights():
        n = 0
        for src, dst, s in ((wgt_hbm, wg_s, S_G), (wut_hbm, wu_s, S_U), (wd_hbm, wd_s, S_D)):
            for r in _rotated_rows(F, 32):
                pltpu.make_async_copy(src.at[pl.ds(r, 32)], dst.at[pl.ds(r, 32)],
                                      w_sem.at[s]).start(priority=n % 2)
                n += 1

    def wait_all(view, s):
        pltpu.make_async_copy(view, view, w_sem.at[s]).wait()

    def start_slot(i, slot):
        h = i // NCH
        row0 = (i % NCH) * T
        for n, (a, b, r0, nr) in enumerate(_kv_pieces()):
            src, dst = ((k_hbm, kbuf), (v_hbm, vbuf))[a]
            pltpu.make_async_copy(src.at[b, h, pl.ds(pl.multiple_of(row0 + r0, 16), nr), :],
                                  dst.at[slot, b, pl.ds(r0, nr), :],
                                  kv_sem.at[slot, a]).start(priority=n % 2)

    def wait_slot(buf, slot, a):
        pltpu.make_async_copy(buf.at[slot], buf.at[slot], kv_sem.at[slot, a]).wait()

    x_cp = pltpu.make_async_copy(x_hbm, x_s, w_sem.at[S_X])
    c_cp = pltpu.make_async_copy(c_hbm, c_s, w_sem.at[S_C])
    wr_cp = pltpu.make_async_copy(wr_hbm, wr_s, w_sem.at[S_WR])
    c_cp.start()
    x_cp.start()
    start_tiles(wmod_hbm, wmod_s, w_sem.at[S_MODA], 0, 2 * D, 16, 1024)
    start_tiles(wq_hbm, wq_s, w_sem.at[S_Q], 0, H * DH, 16, 1024)

    def first_slots(s, carry):
        start_slot(s, s)
        return carry
    lax.fori_loop(0, NBUF, first_slots, 0)
    wr_cp.start()

    c_cp.wait()
    cc = c_s[...].astype(f32)
    sc = (cc * jax.nn.sigmoid(cc)).astype(bf16)
    x_cp.wait()
    x = x_s[...].astype(f32)
    xn = _layernorm(x)
    wait_all(wmod_s.at[:, pl.ds(0, 2 * D)], S_MODA)
    mod_a = jnp.dot(sc, wmod_s[:, 0:2 * D], preferred_element_type=f32)
    h1 = xn * (1.0 + mod_a[:, D:2 * D]) + mod_a[:, 0:D]
    wait_all(wq_s, S_Q)
    q_s[...] = jnp.dot(h1.astype(bf16), wq_s[...], preferred_element_type=f32).astype(bf16)

    scale = (DH ** -0.5) * LOG2E
    row_t = lax.broadcasted_iota(jnp.int32, (B, T), 0)
    row_d = lax.broadcasted_iota(jnp.int32, (B, DH), 0)

    def head_body(h, attn):
        qh = q_s[:, pl.ds(pl.multiple_of(h * DH, DH), DH)]

        def chunk_body(c, carry):
            m, l, acc = carry
            i = h * NCH + c
            slot = i % NBUF
            wait_slot(kbuf, slot, 0)
            s = lax.dot_general(qh, kbuf[slot, 0], NT_DIMS, preferred_element_type=f32)
            for b in range(1, B):
                s_b = lax.dot_general(qh, kbuf[slot, b], NT_DIMS, preferred_element_type=f32)
                s = jnp.where(row_t == b, s_b, s)
            s = s * scale
            m_new = jnp.maximum(m, jnp.max(s, axis=1, keepdims=True))
            alpha = jnp.exp2(m - m_new)
            p = jnp.exp2(s - m_new)
            l = l * alpha + jnp.sum(p, axis=1, keepdims=True)
            pb = p.astype(bf16)
            wait_slot(vbuf, slot, 1)
            o = jnp.dot(pb, vbuf[slot, 0], preferred_element_type=f32)
            for b in range(1, B):
                o_b = jnp.dot(pb, vbuf[slot, b], preferred_element_type=f32)
                o = jnp.where(row_d == b, o_b, o)
            acc = acc * alpha + o

            @pl.when(i + NBUF < NITER)
            def _():
                start_slot(i + NBUF, slot)

            @pl.when(i == 0)
            def _():
                start_tiles(wo_hbm, wo_s, w_sem.at[S_O], 0, D, 32, D)

            @pl.when(i == 1)
            def _():
                start_tiles(wmod_hbm, wmod_s, w_sem.at[S_MODB], 2 * D, 4 * D, 8, 2048)

            @pl.when(i + NBUF == NITER)
            def _():
                start_ffn_weights()
            return m_new, l, acc

        init = (jnp.full((B, 1), -jnp.inf, f32), jnp.zeros((B, 1), f32), jnp.zeros((B, DH), f32))
        _, l, acc = lax.fori_loop(0, NCH, chunk_body, init)
        oh = (acc / l).astype(bf16)

        @pl.when(h == 0)
        def _():
            wait_all(wo_s, S_O)
        wo_h = wo_s[pl.ds(pl.multiple_of(h * DH, DH), DH), :]
        return attn + jnp.dot(oh, wo_h, preferred_element_type=f32)

    attn = lax.fori_loop(0, H, head_body, jnp.zeros((B, D), f32))

    wait_all(wmod_s.at[:, pl.ds(2 * D, 4 * D)], S_MODB)
    mod_b = jnp.dot(sc, wmod_s[:, 2 * D:6 * D], preferred_element_type=f32)
    ga, sb, cb, gb = [mod_b[:, j * D:(j + 1) * D] for j in range(4)]
    x1 = x + ga * attn
    h2 = _layernorm(x1) * (1.0 + cb) + sb
    h2b = h2.astype(bf16)
    wr_cp.wait()
    r = jnp.sum(h2b.astype(f32) * wr_s[...].reshape(1, D).astype(f32), axis=-1, keepdims=True)
    wait_all(wg_s, S_G)
    g = lax.dot_general(h2b, wg_s[...], NT_DIMS, preferred_element_type=f32)
    wait_all(wu_s, S_U)
    u = lax.dot_general(h2b, wu_s[...], NT_DIMS, preferred_element_type=f32)
    a = ((g * jax.nn.sigmoid(g)) * u).astype(bf16)
    wait_all(wd_s, S_D)
    y = jnp.dot(a, wd_s[...], preferred_element_type=f32) * jax.nn.sigmoid(r)
    out = x1 + gb * (h2 + (h2 * 0.0 + y))
    o_s[...] = out.astype(o_s.dtype)
    o_cp = pltpu.make_async_copy(o_s, o_hbm, w_sem.at[S_X])
    o_cp.start()
    o_cp.wait()


@jax.jit
def pallas_adaLN_cond__gqa_block_cached__moe_arch_mod__decode_kernel(
    A_x: jax.Array,
    A_k_cache: jax.Array,
    A_v_cache: jax.Array,
    A_wq: jax.Array,
    A_wo: jax.Array,
    B_x: jax.Array,
    B_w_r: jax.Array,
    B_w_gate: jax.Array,
    B_w_up: jax.Array,
    B_w_down: jax.Array,
    c: jax.Array,
    w_mod: jax.Array,
):
    del B_x
    bf16 = jnp.bfloat16
    hbm = pl.BlockSpec(memory_space=pltpu.HBM)
    out = pl.pallas_call(
        _kernel,
        out_shape=jax.ShapeDtypeStruct((B, D), A_x.dtype),
        in_specs=[hbm] * 11,
        out_specs=hbm,
        scratch_shapes=[
            pltpu.VMEM((NBUF, B, T, DH), bf16),
            pltpu.VMEM((NBUF, B, T, DH), bf16),
            pltpu.VMEM((B, D), bf16),
            pltpu.VMEM((B, D), bf16),
            pltpu.VMEM((D,), bf16),
            pltpu.VMEM((D, H * DH), bf16),
            pltpu.VMEM((H * DH, D), bf16),
            pltpu.VMEM((D, 6 * D), bf16),
            pltpu.VMEM((F, D), bf16),
            pltpu.VMEM((F, D), bf16),
            pltpu.VMEM((F, D), bf16),
            pltpu.VMEM((B, H * DH), bf16),
            pltpu.VMEM((B, D), bf16),
            pltpu.SemaphoreType.DMA((NBUF, 2)),
            pltpu.SemaphoreType.DMA((10,)),
        ],
        compiler_params=pltpu.CompilerParams(
            vmem_limit_bytes=48 * 1024 * 1024,
            disable_bounds_checks=True,
            disable_semaphore_checks=True,
        ),
    )(A_x.reshape(B, D), c, B_w_r, A_k_cache, A_v_cache, A_wq, A_wo, w_mod, B_w_gate.T, B_w_up.T, B_w_down)
    return out.reshape(B, 1, D)
```

```python
import jax
import jax.numpy as jnp
from jax import lax
from jax.experimental import pallas as pl
from jax.experimental.pallas import tpu as pltpu

B, D, H, SK, DH, F = 4, 512, 32, 8192, 128, 1376

T = 2048
NBUF = 2
ROWS = 128
V_SHIFT = 64
NSTREAM = 8
NCH = SK // T
NITER = H * NCH

LOG2E = 1.4426950408889634
NT_DIMS = (((1,), (1,)), ((), ()))

S_X, S_C, S_WR, S_MODA, S_Q, S_O, S_MODB, S_G, S_U, S_D = range(10)


def _kv_pieces():
    pieces = [(1, b, 0, V_SHIFT) for b in range(B)]
    for t in range(T // ROWS):
        pieces += [(0, b, t * ROWS, ROWS) for b in range(B)]
        v_rows = ROWS if (t + 1) * ROWS < T else ROWS - V_SHIFT
        pieces += [(1, b, V_SHIFT + t * ROWS, v_rows) for b in range(B)]
    return pieces


def _rotated_rows(nrows, step):
    n = nrows // step
    seg = -(-n // NSTREAM)
    return [(s * seg + i) * step for i in range(seg) for s in range(NSTREAM) if s * seg + i < n]


def _layernorm(v):
    mean = jnp.mean(v, axis=-1, keepdims=True)
    d = v - mean
    var = jnp.mean(d * d, axis=-1, keepdims=True)
    return d * lax.rsqrt(var + 1e-5)


def _kernel(x_hbm, c_hbm, wr_hbm, k_hbm, v_hbm, wq_hbm, wo_hbm, wmod_hbm, wgt_hbm, wut_hbm, wd_hbm,
            o_hbm,
            kbuf, vbuf, x_s, c_s, wr_s, wq_s, wo_s, wmod_s, wg_s, wu_s, wd_s, q_s, o_s, kv_sem, w_sem):
    f32, bf16 = jnp.float32, jnp.bfloat16

    def start_tiles(src, dst, sem, col0, ncols, pr, pc):
        ncj = ncols // pc
        seg = (src.shape[0] // pr) * ncj // NSTREAM

        def body(j, carry):
            for u in range(NSTREAM):
                idx = u * seg + j
                rows = pl.ds(pl.multiple_of((idx // ncj) * pr, 8), pr)
                cols = pl.ds(pl.multiple_of(col0 + (idx % ncj) * pc, 128), pc)
                pltpu.make_async_copy(src.at[rows, cols], dst.at[rows, cols], sem).start(priority=u % 2)
            return carry
        lax.fori_loop(0, seg, body, 0)

    def start_ffn_weights():
        n = 0
        for src, dst, s in ((wgt_hbm, wg_s, S_G), (wut_hbm, wu_s, S_U), (wd_hbm, wd_s, S_D)):
            for r in _rotated_rows(F, 32):
                pltpu.make_async_copy(src.at[pl.ds(r, 32)], dst.at[pl.ds(r, 32)],
                                      w_sem.at[s]).start(priority=n % 2)
                n += 1

    def wait_all(view, s):
        pltpu.make_async_copy(view, view, w_sem.at[s]).wait()

    def start_slot(i, slot):
        h = i // NCH
        row0 = (i % NCH) * T
        for n, (a, b, r0, nr) in enumerate(_kv_pieces()):
            src, dst = ((k_hbm, kbuf), (v_hbm, vbuf))[a]
            pltpu.make_async_copy(src.at[b, h, pl.ds(pl.multiple_of(row0 + r0, 16), nr), :],
                                  dst.at[slot, b, pl.ds(r0, nr), :],
                                  kv_sem.at[slot, a]).start(priority=n % 2)

    def wait_slot(buf, slot, a):
        pltpu.make_async_copy(buf.at[slot], buf.at[slot], kv_sem.at[slot, a]).wait()

    x_cp = pltpu.make_async_copy(x_hbm, x_s, w_sem.at[S_X])
    c_cp = pltpu.make_async_copy(c_hbm, c_s, w_sem.at[S_C])
    wr_cp = pltpu.make_async_copy(wr_hbm, wr_s, w_sem.at[S_WR])
    c_cp.start()
    x_cp.start()
    start_tiles(wmod_hbm, wmod_s, w_sem.at[S_MODA], 0, 2 * D, 16, 1024)
    start_tiles(wq_hbm, wq_s, w_sem.at[S_Q], 0, H * DH, 16, 1024)
    wr_cp.start()

    c_cp.wait()
    cc = c_s[...].astype(f32)
    sc = (cc * jax.nn.sigmoid(cc)).astype(bf16)
    x_cp.wait()
    x = x_s[...].astype(f32)
    xn = _layernorm(x)
    wait_all(wmod_s.at[:, pl.ds(0, 2 * D)], S_MODA)
    mod_a = jnp.dot(sc, wmod_s[:, 0:2 * D], preferred_element_type=f32)
    h1 = xn * (1.0 + mod_a[:, D:2 * D]) + mod_a[:, 0:D]
    start_slot(0, 0)
    wait_all(wq_s, S_Q)
    q_s[...] = jnp.dot(h1.astype(bf16), wq_s[...], preferred_element_type=f32).astype(bf16)
    for s in range(1, NBUF):
        start_slot(s, s)

    scale = (DH ** -0.5) * LOG2E
    row_t = lax.broadcasted_iota(jnp.int32, (B, T), 0)
    row_d = lax.broadcasted_iota(jnp.int32, (B, DH), 0)

    def head_body(h, attn):
        qh = q_s[:, pl.ds(pl.multiple_of(h * DH, DH), DH)]

        def chunk_body(c, carry):
            m, l, acc = carry
            i = h * NCH + c
            slot = i % NBUF
            wait_slot(kbuf, slot, 0)
            s = lax.dot_general(qh, kbuf[slot, 0], NT_DIMS, preferred_element_type=f32)
            for b in range(1, B):
                s_b = lax.dot_general(qh, kbuf[slot, b], NT_DIMS, preferred_element_type=f32)
                s = jnp.where(row_t == b, s_b, s)
            s = s * scale
            m_new = jnp.maximum(m, jnp.max(s, axis=1, keepdims=True))
            alpha = jnp.exp2(m - m_new)
            p = jnp.exp2(s - m_new)
            l = l * alpha + jnp.sum(p, axis=1, keepdims=True)
            pb = p.astype(bf16)
            wait_slot(vbuf, slot, 1)
            o = jnp.dot(pb, vbuf[slot, 0], preferred_element_type=f32)
            for b in range(1, B):
                o_b = jnp.dot(pb, vbuf[slot, b], preferred_element_type=f32)
                o = jnp.where(row_d == b, o_b, o)
            acc = acc * alpha + o

            @pl.when(i + NBUF < NITER)
            def _():
                start_slot(i + NBUF, slot)

            @pl.when(i == 0)
            def _():
                start_tiles(wo_hbm, wo_s, w_sem.at[S_O], 0, D, 32, D)

            @pl.when(i == 1)
            def _():
                start_tiles(wmod_hbm, wmod_s, w_sem.at[S_MODB], 2 * D, 4 * D, 8, 2048)

            @pl.when(i + NBUF == NITER)
            def _():
                start_ffn_weights()
            return m_new, l, acc

        init = (jnp.full((B, 1), -jnp.inf, f32), jnp.zeros((B, 1), f32), jnp.zeros((B, DH), f32))
        _, l, acc = lax.fori_loop(0, NCH, chunk_body, init)
        oh = (acc / l).astype(bf16)

        @pl.when(h == 0)
        def _():
            wait_all(wo_s, S_O)
        wo_h = wo_s[pl.ds(pl.multiple_of(h * DH, DH), DH), :]
        return attn + jnp.dot(oh, wo_h, preferred_element_type=f32)

    attn = lax.fori_loop(0, H, head_body, jnp.zeros((B, D), f32))

    wait_all(wmod_s.at[:, pl.ds(2 * D, 4 * D)], S_MODB)
    mod_b = jnp.dot(sc, wmod_s[:, 2 * D:6 * D], preferred_element_type=f32)
    ga, sb, cb, gb = [mod_b[:, j * D:(j + 1) * D] for j in range(4)]
    x1 = x + ga * attn
    h2 = _layernorm(x1) * (1.0 + cb) + sb
    h2b = h2.astype(bf16)
    wr_cp.wait()
    r = jnp.sum(h2b.astype(f32) * wr_s[...].reshape(1, D).astype(f32), axis=-1, keepdims=True)
    wait_all(wg_s, S_G)
    g = lax.dot_general(h2b, wg_s[...], NT_DIMS, preferred_element_type=f32)
    wait_all(wu_s, S_U)
    u = lax.dot_general(h2b, wu_s[...], NT_DIMS, preferred_element_type=f32)
    a = ((g * jax.nn.sigmoid(g)) * u).astype(bf16)
    wait_all(wd_s, S_D)
    y = jnp.dot(a, wd_s[...], preferred_element_type=f32) * jax.nn.sigmoid(r)
    out = x1 + gb * (h2 + (h2 * 0.0 + y))
    o_s[...] = out.astype(o_s.dtype)
    o_cp = pltpu.make_async_copy(o_s, o_hbm, w_sem.at[S_X])
    o_cp.start()
    o_cp.wait()


@jax.jit
def pallas_adaLN_cond__gqa_block_cached__moe_arch_mod__decode_kernel(
    A_x: jax.Array,
    A_k_cache: jax.Array,
    A_v_cache: jax.Array,
    A_wq: jax.Array,
    A_wo: jax.Array,
    B_x: jax.Array,
    B_w_r: jax.Array,
    B_w_gate: jax.Array,
    B_w_up: jax.Array,
    B_w_down: jax.Array,
    c: jax.Array,
    w_mod: jax.Array,
):
    del B_x
    bf16 = jnp.bfloat16
    hbm = pl.BlockSpec(memory_space=pltpu.HBM)
    out = pl.pallas_call(
        _kernel,
        out_shape=jax.ShapeDtypeStruct((B, D), A_x.dtype),
        in_specs=[hbm] * 11,
        out_specs=hbm,
        scratch_shapes=[
            pltpu.VMEM((NBUF, B, T, DH), bf16),
            pltpu.VMEM((NBUF, B, T, DH), bf16),
            pltpu.VMEM((B, D), bf16),
            pltpu.VMEM((B, D), bf16),
            pltpu.VMEM((D,), bf16),
            pltpu.VMEM((D, H * DH), bf16),
            pltpu.VMEM((H * DH, D), bf16),
            pltpu.VMEM((D, 6 * D), bf16),
            pltpu.VMEM((F, D), bf16),
            pltpu.VMEM((F, D), bf16),
            pltpu.VMEM((F, D), bf16),
            pltpu.VMEM((B, H * DH), bf16),
            pltpu.VMEM((B, D), bf16),
            pltpu.SemaphoreType.DMA((NBUF, 2)),
            pltpu.SemaphoreType.DMA((10,)),
        ],
        compiler_params=pltpu.CompilerParams(vmem_limit_bytes=48 * 1024 * 1024),
    )(A_x.reshape(B, D), c, B_w_r, A_k_cache, A_v_cache, A_wq, A_wo, w_mod, B_w_gate.T, B_w_up.T, B_w_down)
    return out.reshape(B, 1, D)
```
